```python
import os as _os
_os.environ.setdefault("JAX_PLATFORMS", "cpu")
import jax
import jax.numpy as jnp

def _softmax(x, axis=-1):
    return jax.nn.softmax(x, axis=axis)
def _gelu(x):
    return jax.nn.gelu(x, approximate=True)
def _silu(x):
    return jax.nn.silu(x)
def _sigmoid(x):
    return jax.nn.sigmoid(x)
def _layernorm(x, axis=-1, eps=1e-5):
    m = jnp.mean(x, axis=axis, keepdims=True)
    v = jnp.var(x, axis=axis, keepdims=True)
    return (x - m) / jnp.sqrt(v + eps)
def _scatter_add(tgt, idx, src, axis=0):
    return tgt.at[idx].add(src)
def _segment_sum(src, seg, n):
    return jax.ops.segment_sum(src, seg, n)
class _Rng:
    def __init__(self, key):
        self._k = key
    def _next(self):
        self._k, sub = jax.random.split(self._k)
        return sub
    def normal(self, shape):
        return jax.random.normal(self._next(), shape, dtype=jnp.bfloat16)
    def randint(self, lo, hi, shape):
        return jax.random.randint(self._next(), shape, lo, hi, dtype=jnp.int32)
    def uniform(self, shape, lo=0.0, hi=1.0):
        return jax.random.uniform(self._next(), shape, jnp.bfloat16, lo, hi)
    def permutation(self, n):
        return jax.random.permutation(self._next(), n)


kernel_name = 'sequential_preLN__sliding_block_cached__mixer_channel_mlp__decode'

def setup_inputs():
    _rng = _Rng(jax.random.key(int.from_bytes(__import__("os").urandom(4), "little")))
    _w = (lambda a: (lambda t: t.astype(jnp.bfloat16) if jnp.issubdtype(t.dtype, jnp.floating) else t)(jnp.asarray(a)))
    def _A_setup():
        B, Sq, D = 1, 1, 512
        Hq, Hkv, Sk, Dh = 32, 8, 65536, 128
        assert Hq % Hkv == 0, (Hq, Hkv)
        return {
            "x": _w((lambda *s: _rng.normal(s) * 0.05)(B, Sq, D)),
            "k_cache": _w((lambda *s: _rng.normal(s) * 3.2)(B, Hkv, Sk, Dh)),
            "v_cache": _w((lambda *s: _rng.normal(s) * 0.2)(B, Hkv, Sk, Dh)),
            "wq": _w((lambda *s: _rng.normal(s) * 3.2)(D, Hq * Dh) * (D ** -0.5)),
            "wo": _w((lambda *s: _rng.normal(s) * 0.2)(Hq * Dh, D) * ((Hq * Dh) ** -0.5)),
        }
    _A_in = _A_setup()

    def _B_setup():
        B, S, D, F = 1, 1, 512, 1792
        return {
            "x": _w((lambda *s: _rng.normal(s) * 0.05)(B, S, D)),
            "w1": _w((lambda *s: _rng.normal(s) * 0.2)(D, F) * (D ** -0.5)),
            "b1": _w((lambda *s: _rng.normal(s) * 0.2)(F)),
            "w2": _w((lambda *s: _rng.normal(s) * 0.2)(F, D) * (F ** -0.5)),
            "b2": _w((lambda *s: _rng.normal(s) * 0.05)(D)),
        }
    _B_in = _B_setup()

    return {
        "A_x": _A_in["x"],
        "A_k_cache": _A_in["k_cache"],
        "A_v_cache": _A_in["v_cache"],
        "A_wq": _A_in["wq"],
        "A_wo": _A_in["wo"],
        "B_x": _B_in["x"],
        "B_w1": _B_in["w1"],
        "B_b1": _B_in["b1"],
        "B_w2": _B_in["w2"],
        "B_b2": _B_in["b2"],
    }

def reference(A_x, A_k_cache, A_v_cache, A_wq, A_wo, B_x, B_w1, B_b1, B_w2, B_b2):
    def _A_ref(x, k_cache, v_cache, wq, wo):
        B, Sq, D = x.shape
        Hq, Dh = 32, 128
        Hkv, Sk = k_cache.shape[1], k_cache.shape[2]
        W = min(4096, max(256, Sk // 4))
        rep = Hq // Hkv
        q = (lambda x, *d: x.transpose(*d))((x @ wq).reshape(B, Sq, Hq, Dh), 0, 2, 1, 3)
        k = jnp.repeat(k_cache[:, :, Sk - W:, :], rep, axis=1)
        v = jnp.repeat(v_cache[:, :, Sk - W:, :], rep, axis=1)
        scores = jnp.einsum("bhqd,bhkd->bhqk", q, k) * (Dh ** -0.5)
        p = _softmax(scores, axis=-1)
        o = jnp.einsum("bhqk,bhkd->bhqd", p, v)
        return (lambda x, *d: x.transpose(*d))(o, 0, 2, 1, 3).reshape(B, Sq, Hq * Dh) @ wo

    def _B_ref(x, w1, b1, w2, b2):
        y = _layernorm(x, axis=-1)
        h = _gelu(jnp.einsum("bsd,df->bsf", y, w1) + b1)
        return jnp.einsum("bsf,fd->bsd", h, w2) + b2

    x = A_x
    h = x + _A_ref(_layernorm(x, axis=-1), A_k_cache, A_v_cache, A_wq, A_wo)
    h2 = h + _B_ref(_layernorm(h, axis=-1), B_w1, B_b1, B_w2, B_b2)
    return h2
```

```python
import functools

import jax
import jax.numpy as jnp
from jax import lax
from jax.experimental import pallas as pl
from jax.experimental.pallas import tpu as pltpu

F32 = jnp.float32
BF16 = jnp.bfloat16
D = 512
HQ, HKV, DH = 32, 8, 128
FF = 1792
P = 128


def _r(x):
    return x.astype(BF16).astype(F32)


def _ln(x):
    m = jnp.mean(x, axis=-1, keepdims=True)
    v = jnp.mean(jnp.square(x - m), axis=-1, keepdims=True)
    return _r(_r(x - _r(m)) / _r(jnp.sqrt(_r(_r(v) + 1e-5))))


def make(pace=50, npace=2, qbits=(4, 5, 6, 3), sa=8, tail_groups=(640, 640, 384, 128), **cp):
    rest = [b for b in range(7) if b not in qbits]

    def wpiece(rnd, j):
        s = sum(((j >> i) & 1) << b for i, b in enumerate(qbits))
        t = s
        for i, b in enumerate(rest):
            t = t + (((rnd >> i) & 1) << b)
        return t

    def kern(x_h, k_h, v_h, wq_h, wo_h, w1_h, b1_h, w2_h, b2_h, o_h,
             x_v, kv_v, wq_v, wo_v, w1_v, b1_v, w2_v, b2_v, o_v, q_v, sems):
        sk = k_h.shape[2]
        w = kv_v.shape[0] * P
        S_X, S_B1, S_B2, S_Q, S_O, S_W1, S_W2, S_KV = 0, 1, 2, 3, 4, 5, 6, 6 + len(tail_groups)

        def issue_q(rnd, delay):
            for j in range(16):
                t = wpiece(rnd, j)
                r0 = pl.multiple_of((t >> 1) * 8, 8)
                c0 = pl.multiple_of((t & 1) * 2048, 2048)
                pltpu.make_async_copy(wq_h.at[pl.ds(r0, 8), pl.ds(c0, 2048)],
                                      wq_v.at[pl.ds(r0, 8), pl.ds(c0, 2048)], sems.at[S_Q]).start(priority=j % 2)
                if delay and j % 2:
                    pl.delay(delay)

        def issue_kv(i):
            r0 = pl.multiple_of(sk - w + i * P, P)
            for h in range(HKV):
                pltpu.make_async_copy(k_h.at[0, h, pl.ds(r0, P)], kv_v.at[i, h], sems.at[S_KV + i]).start(priority=0)
                pltpu.make_async_copy(v_h.at[0, h, pl.ds(r0, P)], kv_v.at[i, HKV + h], sems.at[S_KV + i]).start(priority=1)

        def issue_o(rnd, js):
            for j in js:
                r0 = pl.multiple_of(wpiece(rnd, j) * 32, 32)
                pltpu.make_async_copy(wo_h.at[pl.ds(r0, 32)], wo_v.at[pl.ds(r0, 32)], sems.at[S_O]).start(priority=j % 2)

        cx = pltpu.make_async_copy(x_h, x_v, sems.at[S_X])
        cb1 = pltpu.make_async_copy(b1_h, b1_v, sems.at[S_B1])
        cb2 = pltpu.make_async_copy(b2_h, b2_v, sems.at[S_B2])

        lax.fori_loop(0, npace, lambda i, _: issue_q(i, pace), None)
        lax.fori_loop(npace, 8, lambda i, _: issue_q(i, 0), None)
        cx.start(priority=0)
        cb1.start(priority=1)
        cb2.start(priority=0)
        lax.fori_loop(0, 8, lambda i, _: issue_kv(i), None)
        cx.wait()
        x = x_v[0].astype(F32)
        xn = jnp.broadcast_to(_ln(x), (8, D)).astype(BF16)
        pltpu.make_async_copy(wq_v, wq_v, sems.at[S_Q]).wait()
        row = lax.broadcasted_iota(jnp.int32, (8, DH), 0)

        def qproj(g, _):
            issue_kv(8 + g)
            c0 = pl.multiple_of(g * 512, 512)
            q = jnp.dot(xn, wq_v[:, pl.ds(c0, 512)], preferred_element_type=F32)
            r4 = row & 3
            qg = jnp.where(r4 == 0, q[:, 0:128], jnp.where(r4 == 1, q[:, 128:256],
                           jnp.where(r4 == 2, q[:, 256:384], q[:, 384:512])))
            q_v[g] = qg

        lax.fori_loop(0, 8, qproj, None)
        lo = row < 4
        qp = [jnp.where(lo, q_v[2 * p], q_v[2 * p + 1]).astype(BF16) for p in range(4)]
        scale = float(jnp.bfloat16.dtype.type(DH ** -0.5))
        nt = (((1,), (1,)), ((), ()))

        def attn(i, carry):
            @pl.when(i < 16)
            def _():
                issue_kv(16 + i)

            @pl.when((i >= 16) & (i % 2 == 0))
            def _():
                issue_o((i - 16) >> 1, range(16))

            pltpu.make_async_copy(kv_v.at[i], kv_v.at[i], sems.at[S_KV + i]).wait()
            ss = [lax.dot_general(qp[h // 2], kv_v[i, h], nt, preferred_element_type=F32) for h in range(HKV)]
            st = []
            for p in range(4):
                m, l, acc = carry[p]
                s = _r(_r(jnp.where(lo, ss[2 * p], ss[2 * p + 1])) * scale)
                mn = jnp.maximum(m, jnp.max(s, axis=-1, keepdims=True))
                st.append((mn, jnp.exp(m - mn), jnp.exp(s - mn).astype(BF16)))
            os_ = [jnp.dot(st[h // 2][2], kv_v[i, HKV + h], preferred_element_type=F32) for h in range(HKV)]
            out = []
            for p in range(4):
                m, l, acc = carry[p]
                mn, a, e = st[p]
                out.append((mn, a * l + e.astype(F32), a * acc + jnp.where(lo, os_[2 * p], os_[2 * p + 1])))
            return out

        z = jnp.zeros((8, DH), F32)
        init = [(jnp.full((8, DH), -jnp.inf, F32), z, z) for _ in range(4)]
        res = lax.fori_loop(0, w // P, attn, init)
        for p in range(4):
            m, l, acc = res[p]
            q_v[p] = acc / jnp.sum(l, axis=-1, keepdims=True)

        def issue_w1(i, _):
            for j in range(64 // sa):
                r0 = pl.multiple_of((j * sa + i) * 8, 8)
                pltpu.make_async_copy(w1_h.at[pl.ds(r0, 8)], w1_v.at[pl.ds(r0, 8)], sems.at[S_W1]).start(priority=j % 2)

        lax.fori_loop(0, sa, issue_w1, None)
        g0 = 0
        c = 0
        for gi, g in enumerate(tail_groups):
            n = g // 32
            st = 4 if n >= 12 else 1
            for o in range(st):
                for j in range(o, n, st):
                    r0 = g0 + j * 32
                    pltpu.make_async_copy(w2_h.at[pl.ds(r0, 32)], w2_v.at[pl.ds(r0, 32)],
                                          sems.at[S_W2 + gi]).start(priority=c % 2)
                    c += 1
            g0 += g

        pltpu.make_async_copy(wo_v, wo_v, sems.at[S_O]).wait()

        def oproj(p, acc):
            o = q_v[p]
            for j in range(8):
                lhs = jnp.broadcast_to(o[j:j + 1, :], (8, DH)).astype(BF16)
                r0 = pl.multiple_of(p * 1024 + j * 128, 128)
                acc = acc + jnp.dot(lhs, wo_v[pl.ds(r0, 128), :], preferred_element_type=F32)
            return acc

        att = lax.fori_loop(0, 4, oproj, jnp.zeros((8, D), F32))
        h = _r(x + _r(att))
        y = _ln(_ln(h)).astype(BF16)
        cb1.wait()
        cb2.wait()
        pltpu.make_async_copy(w1_v, w1_v, sems.at[S_W1]).wait()
        u = _r(jnp.dot(y, w1_v[...], preferred_element_type=F32))
        u = _r(u + b1_v[...].astype(F32).reshape(1, FF))
        act = jax.nn.gelu(u, approximate=True).astype(BF16)
        acc = h + b2_v[...].astype(F32).reshape(1, D)
        g0 = 0
        for gi, g in enumerate(tail_groups):
            blk = w2_v.at[pl.ds(g0, g)]
            pltpu.make_async_copy(blk, blk, sems.at[S_W2 + gi]).wait()
            acc = acc + jnp.dot(act[:, g0:g0 + g], w2_v[g0:g0 + g, :], preferred_element_type=F32)
            g0 += g
        o_v[0] = acc[0:1].astype(BF16)
        co = pltpu.make_async_copy(o_v, o_h, sems.at[S_X])
        co.start()
        co.wait()

    def f(x, k, v, wq, wo, bx, w1, b1, w2, b2):
        sk = k.shape[2]
        w = min(4096, max(256, sk // 4))
        any_ = pl.BlockSpec(memory_space=pl.ANY)
        return pl.pallas_call(
            kern,
            in_specs=[any_] * 9,
            out_specs=any_,
            out_shape=jax.ShapeDtypeStruct(x.shape, x.dtype),
            scratch_shapes=[
                pltpu.VMEM(x.shape, BF16),
                pltpu.VMEM((w // P, 2 * HKV, P, DH), BF16),
                pltpu.VMEM(wq.shape, BF16),
                pltpu.VMEM(wo.shape, BF16),
                pltpu.VMEM(w1.shape, BF16),
                pltpu.VMEM(b1.shape, BF16),
                pltpu.VMEM(w2.shape, BF16),
                pltpu.VMEM(b2.shape, BF16),
                pltpu.VMEM(x.shape, BF16),
                pltpu.VMEM((8, 8, DH), F32),
                pltpu.SemaphoreType.DMA((6 + len(tail_groups) + w // P,)),
            ],
            compiler_params=pltpu.CompilerParams(
                vmem_limit_bytes=64 * 1024 * 1024,
                disable_bounds_checks=True, disable_semaphore_checks=True, **cp),
        )(x, k, v, wq, wo, w1, b1, w2, b2)

    return f


@jax.jit
def pallas_sequential_preLN__sliding_block_cached__mixer_channel_mlp__decode_kernel(
        A_x, A_k_cache, A_v_cache, A_wq, A_wo, B_x, B_w1, B_b1, B_w2, B_b2):
    return make(qbits=(2, 6, 3, 5))(A_x, A_k_cache, A_v_cache, A_wq, A_wo, B_x, B_w1, B_b1, B_w2, B_b2)
```

```python
import jax
import jax.numpy as jnp
import numpy as np
from jax import lax
import jax.experimental.pallas as pl
import jax.experimental.pallas.tpu as pltpu

F32 = jnp.float32
BF16 = jnp.bfloat16

D, FF = 512, 1792
HQ, HKV, DH = 32, 8, 128
WINDOW = 4096
CHUNK = 256
N_CHUNKS = WINDOW // CHUNK
EPS = 1e-5

LEAD_ON_QUEUE0 = (14, 28, 30)
LEAD_SMALL_AFTER = (2, 6, 10)
KV_ROUND = ((0, 0), (4, 0), (0, 64), (4, 64), (2, 0), (6, 0), (2, 64), (6, 64))
WQ_BITS = (0, 6, 5, 1, 2, 3, 4)
WO_BITS = (6, 0, 5, 2, 1, 3, 4)
W1_STEP = 43
W2_QUEUE0 = (3, 9, 6)
W2_QUEUE1 = ((5, 12, 2, 10), (11, 7, 1, 13), (4, 0, 8))
W2_EARLY_AT = (0, 4)
W2_VPU_GROUPS = (2, 2, 2, 2, 2, 1, 1)


def _round_bf16(x):
    return x.astype(BF16).astype(F32)


def _layernorm(x):
    mean = jnp.mean(x, axis=-1, keepdims=True)
    var = jnp.mean(jnp.square(x - mean), axis=-1, keepdims=True)
    std = _round_bf16(jnp.sqrt(_round_bf16(_round_bf16(var) + EPS)))
    return _round_bf16(_round_bf16(x - _round_bf16(mean)) / std)


def _spread(n, bits):
    out = 0
    for i, b in enumerate(bits):
        out = out + (((n >> i) & 1) << b)
    return out


def _ds(start, size):
    return pl.ds(start if isinstance(start, int) else pl.multiple_of(start, size), size)


def _wait_filled(buf, sem):
    pltpu.make_async_copy(buf, buf, sem).wait()


def _tree_sum(terms):
    while len(terms) > 1:
        terms = [sum(terms[i + 1:i + 2], terms[i]) for i in range(0, len(terms), 2)]
    return terms[0]


def _block_kernel(x_hbm, k_hbm, v_hbm, wq_hbm, wo_hbm, w1_hbm, b1_hbm, w2_hbm, b2_hbm, out_hbm,
                  x_buf, kv_buf, wq_buf, wo_buf, w1_buf, b1_buf, w2_buf, b2_buf, out_buf,
                  q_buf, o_buf, io_sem, bias_sem, wq_sem, w1_sem, kv_sem, wo_sem, w2_sem):
    first_key = k_hbm.shape[2] - WINDOW

    def fetch_wq(rnd, j, queue):
        pos = _spread(rnd, WQ_BITS[3:]) + _spread(j, WQ_BITS[:3])
        part = (slice(None), _ds((pos >> 2) * 8, 8), _ds((pos & 3) * 1024, 1024))
        pltpu.make_async_copy(wq_hbm.at[part], wq_buf.at[part], wq_sem).start(priority=queue)

    def fetch_kv(rnd, j, queue):
        head, row = KV_ROUND[j]
        src = (k_hbm, v_hbm)[queue].at[0, pl.ds(head, 2), _ds(first_key + rnd * 128 + row, 64)]
        dst = kv_buf.at[rnd >> 1, pl.ds(queue * HKV + head, 2), _ds((rnd & 1) * 128 + row, 64)]
        pltpu.make_async_copy(src, dst, kv_sem.at[rnd >> 1]).start(priority=queue)

    wo_head_bits = [b - 3 for b in WO_BITS[:5] if b >= 3]
    wo_buf_bits = [b if b < 3 else 3 + wo_head_bits.index(b - 3) for b in WO_BITS[:5]]

    def fetch_wo(rnd, j):
        pos = _spread(rnd, WO_BITS[3:]) + _spread(j, WO_BITS[:3])
        dst = _spread(rnd, wo_buf_bits[3:]) + _spread(j, wo_buf_bits[:3])
        pltpu.make_async_copy(wo_hbm.at[:, _ds(pos * 16, 16)],
                              wo_buf.at[rnd >> 2, :, _ds(dst * 16, 16)],
                              wo_sem.at[rnd >> 2]).start(priority=1)

    def fetch_w1(n):
        rows = _ds(((n * W1_STEP) & 63) * 8, 8)
        pltpu.make_async_copy(w1_hbm.at[rows], w1_buf.at[rows], w1_sem).start(priority=0)

    def fetch_w2(block, quarter, slot, group, queue):
        pltpu.make_async_copy(w2_hbm.at[_ds(block * 128 + quarter * 32, 32)],
                              w2_buf.at[_ds(slot * 32, 32)],
                              w2_sem.at[group]).start(priority=queue)

    copy_x = pltpu.make_async_copy(x_hbm, x_buf, io_sem)
    copy_b1 = pltpu.make_async_copy(b1_hbm, b1_buf, bias_sem)
    copy_b2 = pltpu.make_async_copy(b2_hbm, b2_buf, bias_sem)

    for n in range(32):
        fetch_wq(n // 8, n % 8, 0 if n in LEAD_ON_QUEUE0 else 1)
        if n in LEAD_SMALL_AFTER:
            (copy_x, copy_b1, copy_b2)[LEAD_SMALL_AFTER.index(n)].start(priority=0)

    def wq_v_round(rnd, _):
        for j in range(8):
            fetch_wq(rnd + 4, j, 0)
            fetch_kv(rnd, j, 1)

    def k_v_round(rnd, _):
        for j in range(8):
            fetch_kv(rnd - 12, j, 0)
            fetch_kv(rnd, j, 1)

    lax.fori_loop(0, 12, wq_v_round, None)
    lax.fori_loop(12, 24, k_v_round, None)

    copy_x.wait()
    x = x_buf[0].astype(F32)
    xn = jnp.broadcast_to(_layernorm(x), (8, D)).astype(BF16)
    _wait_filled(wq_buf, wq_sem)
    sublane = lax.broadcasted_iota(jnp.int32, (8, DH), 0)

    def project_q(g, _):
        k_v_round(24 + g, None)
        cols = _ds(g * 4 * DH, 4 * DH)
        q = (jnp.dot(xn[:, :D // 2], wq_buf[0, :, cols], preferred_element_type=F32)
             + jnp.dot(xn[:, D // 2:], wq_buf[1, :, cols], preferred_element_type=F32))
        rows = q[:, :DH]
        for r in range(1, 4):
            rows = jnp.where((sublane & 3) == r, q[:, r * DH:(r + 1) * DH], rows)
        q_buf[g] = rows

    lax.fori_loop(0, HKV, project_q, None)

    first = sublane < 4
    first_wide = lax.broadcasted_iota(jnp.int32, (8, CHUNK), 0) < 4
    q_pairs = [jnp.where(first, q_buf[2 * p], q_buf[2 * p + 1]).astype(BF16)
               for p in range(HKV // 2)]
    scale = float(np.asarray(DH ** -0.5, dtype=BF16))
    w1_per_round = 8 - len(W2_EARLY_AT)

    def attend(c, state):
        @pl.when(c < 12)
        def _():
            for j in range(8):
                fetch_kv(c + 20, j, 0)
                fetch_wo(c, j)

        @pl.when(c >= 12)
        def _():
            for j in range(8):
                if j in W2_EARLY_AT:
                    i = W2_EARLY_AT.index(j)
                    fetch_w2(W2_QUEUE0[i], c - 12, 4 * i + c - 12, 0, 0)
                else:
                    fetch_w1((c - 12) * w1_per_round + j - sum(e < j for e in W2_EARLY_AT))
                fetch_wo(c, j)

        _wait_filled(kv_buf.at[c], kv_sem.at[c])
        qk = [lax.dot_general(q_pairs[h // 2], kv_buf[c, h], (((1,), (1,)), ((), ())),
                              preferred_element_type=F32) for h in range(HKV)]
        tops, probs = [], []
        for p, (top, _, _) in enumerate(state):
            s = _round_bf16(_round_bf16(jnp.where(first_wide, qk[2 * p], qk[2 * p + 1])) * scale)
            tops.append(jnp.maximum(top, jnp.max(s, axis=-1, keepdims=True)))
            probs.append(jnp.exp(s - tops[p]).astype(BF16))
        pv = [jnp.dot(probs[h // 2], kv_buf[c, HKV + h], preferred_element_type=F32)
              for h in range(HKV)]
        new_state = []
        for p, (top, total, acc) in enumerate(state):
            decay = jnp.exp(top - tops[p])
            e = probs[p].astype(F32)
            new_state.append((tops[p],
                              decay * total + (e[:, :DH] + e[:, DH:]),
                              decay * acc + jnp.where(first, pv[2 * p], pv[2 * p + 1])))
        return new_state

    zeros = jnp.zeros((8, DH), F32)
    lowest = jnp.full((8, 1), float(np.finfo(np.float32).min), F32)
    state = lax.fori_loop(0, N_CHUNKS, attend, [(lowest, zeros, zeros)] * (HKV // 2))
    for p, (_, total, acc) in enumerate(state):
        o_buf[8 * p:8 * p + 8] = acc / jnp.sum(total, axis=-1, keepdims=True)

    mxu_groups = (W2_QUEUE0 + W2_QUEUE1[0], W2_QUEUE1[1])
    mxu_blocks = mxu_groups[0] + mxu_groups[1]
    vpu_parts = [(b, quarter) for quarter in range(4) for b in W2_QUEUE1[2]]
    vpu_group = [g for g, n in enumerate(W2_VPU_GROUPS) for _ in range(n)]
    queue0 = [(fetch_w1, n) for n in range(4 * w1_per_round, 64)]
    queue0 += [(fetch_w2, b, quarter, 4 * mxu_blocks.index(b) + quarter, 0, 0)
               for quarter in range(4) for b in W2_QUEUE0[len(W2_EARLY_AT):]]
    queue1 = [(fetch_w2, b, quarter, 4 * mxu_blocks.index(b) + quarter, g, 1)
              for g in range(2) for quarter in range(4) for b in W2_QUEUE1[g]]
    queue1 += [(fetch_w2, b, quarter, 4 * len(mxu_blocks) + i, 2 + vpu_group[i], 1)
               for i, (b, quarter) in enumerate(vpu_parts)]
    for pair in zip(queue0, queue1, strict=True):
        for fetch, *where in pair:
            fetch(*where)

    def project_o(p, acc):
        _wait_filled(wo_buf.at[p], wo_sem.at[p])
        for half in range(2):
            for i in range(4):
                head = (half * (HQ // 2) + _spread(p, [b - 3 for b in WO_BITS[5:]])
                        + _spread(i, wo_head_bits))
                o = jnp.broadcast_to(o_buf[pl.ds(head, 1), :], (8, DH)).astype(BF16)
                acc = acc + jnp.dot(o, wo_buf[p, half, i * DH:(i + 1) * DH, :],
                                    preferred_element_type=F32)
        return acc

    attn = lax.fori_loop(0, 4, project_o, jnp.zeros((8, D), F32))
    h = _round_bf16(x + _round_bf16(attn))

    y = _layernorm(_layernorm(h)).astype(BF16)
    copy_b1.wait()
    copy_b2.wait()
    _wait_filled(w1_buf, w1_sem)
    pre = _round_bf16(jnp.dot(y, w1_buf[...], preferred_element_type=F32))
    pre = _round_bf16(pre + b1_buf[...].astype(F32).reshape(1, FF))
    act = _round_bf16(jax.nn.gelu(pre, approximate=True))

    acc = h + b2_buf[...].astype(F32).reshape(1, D)
    row = 0
    for g, blocks in enumerate(mxu_groups):
        rows = pl.ds(row, 128 * len(blocks))
        _wait_filled(w2_buf.at[rows], w2_sem.at[g])
        if g == 0:
            act_t = {b: jnp.concatenate([act[:, b * 128:(b + 1) * 128]] * 16, axis=0).T
                     for b in W2_QUEUE1[2]}
        lhs = jnp.concatenate([act[:, b * 128:(b + 1) * 128] for b in blocks], axis=1)
        acc = acc + jnp.dot(lhs.astype(BF16), w2_buf[rows, :], preferred_element_type=F32)
        row += 128 * len(blocks)

    acc = jnp.where(lax.broadcasted_iota(jnp.int32, (8, D), 0) == 0, acc, 0.0)
    done = 0
    for g, n in enumerate(W2_VPU_GROUPS):
        _wait_filled(w2_buf.at[pl.ds(row, 32 * n)], w2_sem.at[2 + g])
        terms = [acc]
        for b, quarter in vpu_parts[done:done + n]:
            for r in range(quarter * 32, quarter * 32 + 32, 8):
                a = jnp.concatenate([act_t[b][r:r + 8, :]] * (D // 128), axis=1)
                terms.append(w2_buf[row:row + 8, :].astype(F32) * a)
                row += 8
        acc = _tree_sum(terms)
        done += n

    out_buf[0] = jnp.sum(acc, axis=0, keepdims=True).astype(out_buf.dtype)
    copy_out = pltpu.make_async_copy(out_buf, out_hbm, io_sem)
    copy_out.start()
    copy_out.wait()


@jax.jit
def pallas_sequential_preLN__sliding_block_cached__mixer_channel_mlp__decode_kernel(
    A_x: jax.Array,
    A_k_cache: jax.Array,
    A_v_cache: jax.Array,
    A_wq: jax.Array,
    A_wo: jax.Array,
    B_x: jax.Array,
    B_w1: jax.Array,
    B_b1: jax.Array,
    B_w2: jax.Array,
    B_b2: jax.Array,
):
    del B_x
    cache_len = A_k_cache.shape[2]
    assert A_x.shape == (1, 1, D) and B_w1.shape == (D, FF) and B_w2.shape == (FF, D)
    assert A_k_cache.shape == A_v_cache.shape == (1, HKV, cache_len, DH)
    assert min(4096, max(256, cache_len // 4)) == WINDOW and cache_len % 64 == 0

    wq = A_wq.reshape(2, D // 2, HQ * DH)
    wo = A_wo.reshape(2, HQ * DH // 2, D)

    in_hbm = pl.BlockSpec(memory_space=pl.ANY)
    return pl.pallas_call(
        _block_kernel,
        in_specs=[in_hbm] * 9,
        out_specs=in_hbm,
        out_shape=jax.ShapeDtypeStruct(A_x.shape, A_x.dtype),
        scratch_shapes=[
            pltpu.VMEM(A_x.shape, A_x.dtype),
            pltpu.VMEM((N_CHUNKS, 2 * HKV, CHUNK, DH), A_k_cache.dtype),
            pltpu.VMEM(wq.shape, wq.dtype),
            pltpu.VMEM((4, 2, 4 * DH, D), wo.dtype),
            pltpu.VMEM(B_w1.shape, B_w1.dtype),
            pltpu.VMEM(B_b1.shape, B_b1.dtype),
            pltpu.VMEM(B_w2.shape, B_w2.dtype),
            pltpu.VMEM(B_b2.shape, B_b2.dtype),
            pltpu.VMEM(A_x.shape, A_x.dtype),
            pltpu.VMEM((HKV, 8, DH), F32),
            pltpu.VMEM((HQ, DH), F32),
            pltpu.SemaphoreType.DMA,
            pltpu.SemaphoreType.DMA,
            pltpu.SemaphoreType.DMA,
            pltpu.SemaphoreType.DMA,
            pltpu.SemaphoreType.DMA((N_CHUNKS,)),
            pltpu.SemaphoreType.DMA((4,)),
            pltpu.SemaphoreType.DMA((2 + len(W2_VPU_GROUPS),)),
        ],
        compiler_params=pltpu.CompilerParams(
            vmem_limit_bytes=48 * 1024 * 1024,
            disable_bounds_checks=True,
            disable_semaphore_checks=True,
        ),
    )(A_x, A_k_cache, A_v_cache, wq, wo, B_w1, B_b1, B_w2, B_b2)
```

```python
import jax
import jax.numpy as jnp
import numpy as np
from jax import lax
import jax.experimental.pallas as pl
import jax.experimental.pallas.tpu as pltpu

F32 = jnp.float32
BF16 = jnp.bfloat16

D, FF = 512, 1792
HQ, HKV, DH = 32, 8, 128
WINDOW = 4096
CHUNK = 256
N_CHUNKS = WINDOW // CHUNK
EPS = 1e-5

LEAD_ON_QUEUE0 = (9, 28, 30)
LEAD_SMALL_AFTER = (0, 3, 6)
KV_ROUND = ((0, 0), (0, 64), (4, 0), (4, 64), (2, 0), (2, 64), (6, 0), (6, 64))
WQ_BITS = (0, 6, 5, 1, 2, 3, 4)
WO_BITS = (0, 6, 5, 2, 1, 3, 4)
W1_STEP = 43
W2_QUEUE0 = (3, 10, 6)
W2_QUEUE1 = ((5, 9, 11, 12), (2, 1, 7, 13), (4, 0, 8))
W2_EARLY_AT = (2, 6)
W2_VPU_GROUPS = (2, 2, 2, 2, 2, 1, 1)

SEM_IO, SEM_BIAS, SEM_WQ, SEM_W1, SEM_WO = range(5)
SEM_KV = SEM_WO + 4
SEM_W2 = SEM_KV + N_CHUNKS


def _round_bf16(x):
    return x.astype(BF16).astype(F32)


def _layernorm(x):
    mean = jnp.mean(x, axis=-1, keepdims=True)
    var = jnp.mean(jnp.square(x - mean), axis=-1, keepdims=True)
    std = _round_bf16(jnp.sqrt(_round_bf16(_round_bf16(var) + EPS)))
    return _round_bf16(_round_bf16(x - _round_bf16(mean)) / std)


def _spread(n, bits):
    out = 0
    for i, b in enumerate(bits):
        out = out + (((n >> i) & 1) << b)
    return out


def _ds(start, size):
    return pl.ds(start if isinstance(start, int) else pl.multiple_of(start, size), size)


def _wait_filled(buf, sem):
    pltpu.make_async_copy(buf, buf, sem).wait()


def _tree_sum(terms):
    while len(terms) > 1:
        terms = [sum(terms[i + 1:i + 2], terms[i]) for i in range(0, len(terms), 2)]
    return terms[0]


def _block_kernel(x_hbm, k_hbm, v_hbm, wq_hbm, wo_hbm, w1_hbm, b1_hbm, w2_hbm, b2_hbm, out_hbm,
                  x_buf, kv_buf, wq_buf, wo_buf, w1_buf, b1_buf, w2_buf, b2_buf, out_buf,
                  q_buf, o_buf, sems):
    first_key = k_hbm.shape[2] - WINDOW

    def fetch_wq(rnd, j, queue):
        pos = _spread(rnd, WQ_BITS[3:]) + _spread(j, WQ_BITS[:3])
        part = (slice(None), _ds((pos >> 2) * 8, 8), _ds((pos & 3) * 1024, 1024))
        pltpu.make_async_copy(wq_hbm.at[part], wq_buf.at[part],
                              sems.at[SEM_WQ]).start(priority=queue)

    def fetch_kv(rnd, j, queue):
        head, row = KV_ROUND[j]
        src = (k_hbm, v_hbm)[queue].at[0, pl.ds(head, 2), _ds(first_key + rnd * 128 + row, 64)]
        dst = kv_buf.at[rnd >> 1, pl.ds(queue * HKV + head, 2), _ds((rnd & 1) * 128 + row, 64)]
        pltpu.make_async_copy(src, dst, sems.at[SEM_KV + (rnd >> 1)]).start(priority=queue)

    wo_head_bits = [b - 3 for b in WO_BITS[:5] if b >= 3]
    wo_buf_bits = [b if b < 3 else 3 + wo_head_bits.index(b - 3) for b in WO_BITS[:5]]

    def fetch_wo(rnd, j):
        pos = _spread(rnd, WO_BITS[3:]) + _spread(j, WO_BITS[:3])
        dst = _spread(rnd, wo_buf_bits[3:]) + _spread(j, wo_buf_bits[:3])
        pltpu.make_async_copy(wo_hbm.at[:, _ds(pos * 16, 16)],
                              wo_buf.at[rnd >> 2, :, _ds(dst * 16, 16)],
                              sems.at[SEM_WO + (rnd >> 2)]).start(priority=1)

    def fetch_w1(n):
        rows = _ds(((n * W1_STEP) & 63) * 8, 8)
        pltpu.make_async_copy(w1_hbm.at[rows], w1_buf.at[rows], sems.at[SEM_W1]).start(priority=0)

    def fetch_w2(block, quarter, slot, group, queue):
        pltpu.make_async_copy(w2_hbm.at[_ds(block * 128 + quarter * 32, 32)],
                              w2_buf.at[_ds(slot * 32, 32)],
                              sems.at[SEM_W2 + group]).start(priority=queue)

    copy_x = pltpu.make_async_copy(x_hbm, x_buf, sems.at[SEM_IO])
    copy_b1 = pltpu.make_async_copy(b1_hbm, b1_buf, sems.at[SEM_BIAS])
    copy_b2 = pltpu.make_async_copy(b2_hbm, b2_buf, sems.at[SEM_BIAS])

    for n in range(32):
        fetch_wq(n // 8, n % 8, 0 if n in LEAD_ON_QUEUE0 else 1)
        if n in LEAD_SMALL_AFTER:
            (copy_x, copy_b1, copy_b2)[LEAD_SMALL_AFTER.index(n)].start(priority=0)

    def wq_v_round(rnd, _):
        for j in range(8):
            fetch_wq(rnd + 4, j, 0)
            fetch_kv(rnd, j, 1)

    def k_v_round(rnd, _):
        for j in range(8):
            fetch_kv(rnd - 12, j, 0)
            fetch_kv(rnd, j, 1)

    lax.fori_loop(0, 12, wq_v_round, None)
    lax.fori_loop(12, 24, k_v_round, None)

    copy_x.wait()
    x = x_buf[0].astype(F32)
    xn = jnp.broadcast_to(_layernorm(x), (8, D)).astype(BF16)
    _wait_filled(wq_buf, sems.at[SEM_WQ])
    sublane = lax.broadcasted_iota(jnp.int32, (8, DH), 0)

    def project_q(g, _):
        k_v_round(24 + g, None)
        cols = _ds(g * 4 * DH, 4 * DH)
        q = (jnp.dot(xn[:, :D // 2], wq_buf[0, :, cols], preferred_element_type=F32)
             + jnp.dot(xn[:, D // 2:], wq_buf[1, :, cols], preferred_element_type=F32))
        rows = q[:, :DH]
        for r in range(1, 4):
            rows = jnp.where((sublane & 3) == r, q[:, r * DH:(r + 1) * DH], rows)
        q_buf[g] = rows

    lax.fori_loop(0, HKV, project_q, None)

    first = sublane < 4
    first_wide = lax.broadcasted_iota(jnp.int32, (8, CHUNK), 0) < 4
    q_pairs = [jnp.where(first, q_buf[2 * p], q_buf[2 * p + 1]).astype(BF16)
               for p in range(HKV // 2)]
    scale = float(np.asarray(DH ** -0.5, dtype=BF16))
    w1_per_round = 8 - len(W2_EARLY_AT)

    def attend(c, state):
        @pl.when(c < 12)
        def _():
            for j in range(8):
                fetch_kv(c + 20, j, 0)
                fetch_wo(c, j)

        @pl.when(c >= 12)
        def _():
            for j in range(8):
                if j in W2_EARLY_AT:
                    i = W2_EARLY_AT.index(j)
                    fetch_w2(W2_QUEUE0[i], c - 12, 4 * i + c - 12, 0, 0)
                else:
                    fetch_w1((c - 12) * w1_per_round + j - sum(e < j for e in W2_EARLY_AT))
                fetch_wo(c, j)

        _wait_filled(kv_buf.at[c], sems.at[SEM_KV + c])
        qk = [lax.dot_general(q_pairs[h // 2], kv_buf[c, h], (((1,), (1,)), ((), ())),
                              preferred_element_type=F32) for h in range(HKV)]
        tops, probs = [], []
        for p, (top, _, _) in enumerate(state):
            s = _round_bf16(_round_bf16(jnp.where(first_wide, qk[2 * p], qk[2 * p + 1])) * scale)
            tops.append(jnp.maximum(top, jnp.max(s, axis=-1, keepdims=True)))
            probs.append(jnp.exp(s - tops[p]).astype(BF16))
        pv = [jnp.dot(probs[h // 2], kv_buf[c, HKV + h], preferred_element_type=F32)
              for h in range(HKV)]
        new_state = []
        for p, (top, total, acc) in enumerate(state):
            decay = jnp.exp(top - tops[p])
            e = probs[p].astype(F32)
            new_state.append((tops[p],
                              decay * total + (e[:, :DH] + e[:, DH:]),
                              decay * acc + jnp.where(first, pv[2 * p], pv[2 * p + 1])))
        return new_state

    zeros = jnp.zeros((8, DH), F32)
    lowest = jnp.full((8, 1), float(np.finfo(np.float32).min), F32)
    state = lax.fori_loop(0, N_CHUNKS, attend, [(lowest, zeros, zeros)] * (HKV // 2))
    for p, (_, total, acc) in enumerate(state):
        o_buf[8 * p:8 * p + 8] = acc / jnp.sum(total, axis=-1, keepdims=True)

    mxu_groups = (W2_QUEUE0 + W2_QUEUE1[0], W2_QUEUE1[1])
    mxu_blocks = mxu_groups[0] + mxu_groups[1]
    vpu_parts = [(b, quarter) for quarter in range(4) for b in W2_QUEUE1[2]]
    vpu_group = [g for g, n in enumerate(W2_VPU_GROUPS) for _ in range(n)]
    queue0 = [(fetch_w1, n) for n in range(4 * w1_per_round, 64)]
    queue0 += [(fetch_w2, b, quarter, 4 * mxu_blocks.index(b) + quarter, 0, 0)
               for quarter in range(4) for b in W2_QUEUE0[len(W2_EARLY_AT):]]
    queue1 = [(fetch_w2, b, quarter, 4 * mxu_blocks.index(b) + quarter, g, 1)
              for g in range(2) for quarter in range(4) for b in W2_QUEUE1[g]]
    queue1 += [(fetch_w2, b, quarter, 4 * len(mxu_blocks) + i, 2 + vpu_group[i], 1)
               for i, (b, quarter) in enumerate(vpu_parts)]
    for pair in zip(queue0, queue1, strict=True):
        for fetch, *where in pair:
            fetch(*where)

    def project_o(p, acc):
        _wait_filled(wo_buf.at[p], sems.at[SEM_WO + p])
        for half in range(2):
            for i in range(4):
                head = (half * (HQ // 2) + _spread(p, [b - 3 for b in WO_BITS[5:]])
                        + _spread(i, wo_head_bits))
                o = jnp.broadcast_to(o_buf[pl.ds(head, 1), :], (8, DH)).astype(BF16)
                acc = acc + jnp.dot(o, wo_buf[p, half, i * DH:(i + 1) * DH, :],
                                    preferred_element_type=F32)
        return acc

    attn = lax.fori_loop(0, 4, project_o, jnp.zeros((8, D), F32))
    h = _round_bf16(x + _round_bf16(attn))

    y = _layernorm(_layernorm(h)).astype(BF16)
    copy_b1.wait()
    copy_b2.wait()
    _wait_filled(w1_buf, sems.at[SEM_W1])
    pre = _round_bf16(jnp.dot(y, w1_buf[...], preferred_element_type=F32))
    pre = _round_bf16(pre + b1_buf[...].astype(F32).reshape(1, FF))
    act = _round_bf16(jax.nn.gelu(pre, approximate=True))

    acc = h + b2_buf[...].astype(F32).reshape(1, D)
    row = 0
    for g, blocks in enumerate(mxu_groups):
        rows = pl.ds(row, 128 * len(blocks))
        _wait_filled(w2_buf.at[rows], sems.at[SEM_W2 + g])
        if g == 0:
            act_t = {b: jnp.concatenate([act[:, b * 128:(b + 1) * 128]] * 16, axis=0).T
                     for b in W2_QUEUE1[2]}
        lhs = jnp.concatenate([act[:, b * 128:(b + 1) * 128] for b in blocks], axis=1)
        acc = acc + jnp.dot(lhs.astype(BF16), w2_buf[rows, :], preferred_element_type=F32)
        row += 128 * len(blocks)

    acc = jnp.where(lax.broadcasted_iota(jnp.int32, (8, D), 0) == 0, acc, 0.0)
    done = 0
    for g, n in enumerate(W2_VPU_GROUPS):
        _wait_filled(w2_buf.at[pl.ds(row, 32 * n)], sems.at[SEM_W2 + 2 + g])
        terms = [acc]
        for b, quarter in vpu_parts[done:done + n]:
            for r in range(quarter * 32, quarter * 32 + 32, 8):
                a = jnp.concatenate([act_t[b][r:r + 8, :]] * (D // 128), axis=1)
                terms.append(w2_buf[row:row + 8, :].astype(F32) * a)
                row += 8
        acc = _tree_sum(terms)
        done += n

    out_buf[0] = jnp.sum(acc, axis=0, keepdims=True).astype(out_buf.dtype)
    copy_out = pltpu.make_async_copy(out_buf, out_hbm, sems.at[SEM_IO])
    copy_out.start()
    copy_out.wait()


@jax.jit
def pallas_sequential_preLN__sliding_block_cached__mixer_channel_mlp__decode_kernel(
    A_x: jax.Array,
    A_k_cache: jax.Array,
    A_v_cache: jax.Array,
    A_wq: jax.Array,
    A_wo: jax.Array,
    B_x: jax.Array,
    B_w1: jax.Array,
    B_b1: jax.Array,
    B_w2: jax.Array,
    B_b2: jax.Array,
):
    del B_x
    cache_len = A_k_cache.shape[2]
    assert A_x.shape == (1, 1, D) and B_w1.shape == (D, FF) and B_w2.shape == (FF, D)
    assert A_k_cache.shape == A_v_cache.shape == (1, HKV, cache_len, DH)
    assert min(4096, max(256, cache_len // 4)) == WINDOW and cache_len % 64 == 0

    wq = A_wq.reshape(2, D // 2, HQ * DH)
    wo = A_wo.reshape(2, HQ * DH // 2, D)

    in_hbm = pl.BlockSpec(memory_space=pl.ANY)
    return pl.pallas_call(
        _block_kernel,
        in_specs=[in_hbm] * 9,
        out_specs=in_hbm,
        out_shape=jax.ShapeDtypeStruct(A_x.shape, A_x.dtype),
        scratch_shapes=[
            pltpu.VMEM(A_x.shape, A_x.dtype),
            pltpu.VMEM((N_CHUNKS, 2 * HKV, CHUNK, DH), A_k_cache.dtype),
            pltpu.VMEM(wq.shape, wq.dtype),
            pltpu.VMEM((4, 2, 4 * DH, D), wo.dtype),
            pltpu.VMEM(B_w1.shape, B_w1.dtype),
            pltpu.VMEM(B_b1.shape, B_b1.dtype),
            pltpu.VMEM(B_w2.shape, B_w2.dtype),
            pltpu.VMEM(B_b2.shape, B_b2.dtype),
            pltpu.VMEM(A_x.shape, A_x.dtype),
            pltpu.VMEM((HKV, 8, DH), F32),
            pltpu.VMEM((HQ, DH), F32),
            pltpu.SemaphoreType.DMA((SEM_W2 + 2 + len(W2_VPU_GROUPS),)),
        ],
        compiler_params=pltpu.CompilerParams(
            vmem_limit_bytes=48 * 1024 * 1024,
            disable_bounds_checks=True,
            disable_semaphore_checks=True,
        ),
    )(A_x, A_k_cache, A_v_cache, wq, wo, B_w1, B_b1, B_w2, B_b2)
```
